```python
import jax
import jax.numpy as jnp

def _softmax(x, axis=-1):
    return jax.nn.softmax(x, axis=axis)
def _gelu(x):
    return jax.nn.gelu(x, approximate=True)
def _silu(x):
    return jax.nn.silu(x)
def _sigmoid(x):
    return jax.nn.sigmoid(x)
def _layernorm(x, axis=-1, eps=1e-5):
    m = jnp.mean(x, axis=axis, keepdims=True)
    v = jnp.var(x, axis=axis, keepdims=True)
    return (x - m) / jnp.sqrt(v + eps)
def _scatter_add(tgt, idx, src, axis=0):
    return tgt.at[idx].add(src)
def _segment_sum(src, seg, n):
    return jax.ops.segment_sum(src, seg, n)
class _Rng:
    def __init__(self, key):
        self._k = key
    def _next(self):
        self._k, sub = jax.random.split(self._k)
        return sub
    def normal(self, shape):
        return jax.random.normal(self._next(), shape, dtype=jnp.bfloat16)
    def randint(self, lo, hi, shape):
        return jax.random.randint(self._next(), shape, lo, hi, dtype=jnp.int32)
    def uniform(self, shape, lo=0.0, hi=1.0):
        return jax.random.uniform(self._next(), shape, jnp.bfloat16, lo, hi)
    def permutation(self, n):
        return jax.random.permutation(self._next(), n)


kernel_name = 'concat_heads__compressed_kv_cla__mha_block_cached__decode'

def setup_inputs():
    _rng = _Rng(jax.random.key(int.from_bytes(__import__("os").urandom(4), "little")))
    _w = (lambda a: (lambda t: t.astype(jnp.bfloat16) if jnp.issubdtype(t.dtype, jnp.floating) else t)(jnp.asarray(a)))
    def _A_setup():
        B, H, Sq, Sk, D, M = 4, 32, 1, 4096, 128, 512
        Dc = 4 * D
        return {
            "x": _w((lambda *s: _rng.normal(s) * 0.05)(B, Sq, M)),
            "c_kv": _w((lambda *s: _rng.normal(s) * 0.05)(B, Sk, Dc)),
            "w_q": _w((lambda *s: _rng.normal(s) * 0.05)(M, H, D) * (M ** -0.5)),
            "w_uk": _w((lambda *s: _rng.normal(s) * 0.05)(Dc, H, D) * (Dc ** -0.5)),
            "w_uv": _w((lambda *s: _rng.normal(s) * 0.05)(Dc, H, D) * (Dc ** -0.5)),
            "w_o": _w((lambda *s: _rng.normal(s) * 0.05)(H, D, M) * ((H * D) ** -0.5)),
        }
    _A_in = _A_setup()

    def _B_setup():
        B, Sq, D = 4, 1, 512
        H, Sk, Dh = 32, 4096, 128
        return {
            "x": _w((lambda *s: _rng.normal(s) * 0.05)(B, Sq, D)),
            "k_cache": _w((lambda *s: _rng.normal(s) * 0.05)(B, H, Sk, Dh)),
            "v_cache": _w((lambda *s: _rng.normal(s) * 0.05)(B, H, Sk, Dh)),
            "wq": _w((lambda *s: _rng.normal(s) * 0.05)(D, H * Dh) * (D ** -0.5)),
            "wo": _w((lambda *s: _rng.normal(s) * 0.05)(H * Dh, D) * ((H * Dh) ** -0.5)),
        }
    _B_in = _B_setup()

    return {
        "A_x": _A_in["x"],
        "A_c_kv": _A_in["c_kv"],
        "A_w_q": _A_in["w_q"],
        "A_w_uk": _A_in["w_uk"],
        "A_w_uv": _A_in["w_uv"],
        "A_w_o": _A_in["w_o"],
        "B_x": _B_in["x"],
        "B_k_cache": _B_in["k_cache"],
        "B_v_cache": _B_in["v_cache"],
        "B_wq": _B_in["wq"],
        "B_wo": _B_in["wo"],
    }

def reference(A_x, A_c_kv, A_w_q, A_w_uk, A_w_uv, A_w_o, B_x, B_k_cache, B_v_cache, B_wq, B_wo):
    def _A_ref(x, c_kv, w_q, w_uk, w_uv, w_o):
        B, Sq, M = x.shape[0], x.shape[1], x.shape[2]
        Sk = c_kv.shape[1]
        H, D = w_q.shape[1], w_q.shape[2]
        q = jnp.einsum("bqm,mhd->bhqd", x, w_q)
        k = jnp.einsum("bkc,chd->bhkd", c_kv, w_uk)
        v = jnp.einsum("bkc,chd->bhkd", c_kv, w_uv)
        scores = jnp.einsum("bhqd,bhkd->bhqk", q, k) * (D ** -0.5)
        off = Sk - Sq
        qi = jnp.arange(Sq)[:, None]
        kj = jnp.arange(Sk)[None, :]
        cmask = kj <= (qi + off)
        scores = jnp.where(cmask[None, None], scores, -1e9)
        p = _softmax(scores, axis=-1)
        ctx = jnp.einsum("bhqk,bhkd->bhqd", p, v)
        return jnp.einsum("bhqd,hdm->bqm", ctx, w_o)

    def _B_ref(x, k_cache, v_cache, wq, wo):
        B, Sq, D = x.shape
        H, Dh = 32, 128
        q = (lambda x, *d: x.transpose(*d))((x @ wq).reshape(B, Sq, H, Dh), 0, 2, 1, 3)
        scores = jnp.einsum("bhqd,bhkd->bhqk", q, k_cache) * (Dh ** -0.5)
        p = _softmax(scores, axis=-1)
        o = jnp.einsum("bhqk,bhkd->bhqd", p, v_cache)
        return (lambda x, *d: x.transpose(*d))(o, 0, 2, 1, 3).reshape(B, Sq, H * Dh) @ wo

    a = _A_ref(A_x, A_c_kv, A_w_q, A_w_uk, A_w_uv, A_w_o)
    b = _B_ref(B_x, B_k_cache, B_v_cache, B_wq, B_wo)
    return jnp.concatenate([a, b], axis=-1)
```

```python
import functools

import jax
import jax.numpy as jnp
from jax import lax
import jax.experimental.pallas as pl
import jax.experimental.pallas.tpu as pltpu

F32 = jnp.float32
BF16 = jnp.bfloat16
NT = (((1,), (1,)), ((), ()))

NB, NH, SK, HD, DM = 4, 32, 4096, 128, 512
KR = 1024
NR = SK // KR
AHEAD = 2
PARTS_128 = (144,) * 6 + (160,)
PARTS_512 = (48, 48, 32, 48, 48, 32)
MIB = 1 << 20
LEAD_BYTES = 4 * MIB


def _offsets(parts):
    out, o = [], 0
    for p in parts:
        out.append((o, p))
        o += p
    return out


def _kernel(ax_hbm, ckv_hbm, wq_hbm, wuk_hbm, wuv_hbm, wo_hbm, bx_hbm, k_hbm, v_hbm, bwq_hbm, bwo_hbm,
            out_ref,
            ax_v, bx_v, ckv_v, wq_v, wuk_v, wuv_v, wo_v, bwq_v, bwo_v, k_v, v_v,
            e_v, r_v, qa_v, sa_v, pa_v, cc_v, qb_v, sb_v, pb_v,
            x_sem, u_sem, bwo_sem, k_sem, v_sem):
    scale = HD ** -0.5

    def wait_all(dst, sem):
        pltpu.make_async_copy(dst, dst, sem).wait()

    def rows_group(src, dst, sem, base, stream_rows, n_streams, off, size):
        def start():
            for s in range(n_streams):
                r0 = base + s * stream_rows + off
                pltpu.make_async_copy(src.at[pl.ds(r0, size)], dst.at[pl.ds(r0, size)], sem).start(priority=s % 2)
        return n_streams * size * src.shape[1] * 2, start

    def bwq_group(sem, r0):
        def start():
            for c in range(8):
                sl = (pl.ds(r0 + 16 * (c // 4), 16), pl.ds((c % 4) * 1024, 1024))
                pltpu.make_async_copy(bwq_hbm.at[sl], bwq_v.at[sl], sem).start(priority=c % 2)
        return 8 * 16 * 1024 * 2, start

    def cache_chunk(src, dst, sem, h, r, b, off, size, priority):
        row = (b * NH + h) * SK + r * KR + off
        if not isinstance(row, int):
            row = pl.multiple_of(row, 16)
        pltpu.make_async_copy(src.at[pl.ds(row, size)], dst.at[r, b, pl.ds(off, size)], sem.at[r]).start(priority=priority)

    def start_kv(hk, hv, r, parts):
        for off, size in parts:
            for b in range(NB):
                if hk is not None:
                    cache_chunk(k_hbm, k_v, k_sem, hk, r, b, off, size, 0 if hv is not None else b % 2)
                if hv is not None:
                    cache_chunk(v_hbm, v_v, v_sem, hv, r, b, off, size, 1 if hk is not None else b % 2)

    def k0_group(r, i):
        def start():
            off, size = _offsets(PARTS_128)[i]
            for b in range(NB):
                cache_chunk(k_hbm, k_v, k_sem, 0, r, b, off, size, 0)
                if i < len(PARTS_512):
                    o2, s2 = _offsets(PARTS_512)[i]
                    r0 = r * 1024 + b * 256 + o2
                    pltpu.make_async_copy(bwo_hbm.at[pl.ds(r0, s2)], bwo_v.at[pl.ds(r0, s2)], bwo_sem).start(priority=1)
        return 2 * MIB // len(PARTS_128), start

    stream, unit_end, unit_dst = [], [], []

    def add_unit(groups, dst):
        stream.extend(groups)
        unit_end.append(sum(g[0] for g in stream))
        unit_dst.append(dst)
        return len(unit_end) - 1

    def add_rows_unit(src, dst, base, rows, parts):
        sem = u_sem.at[len(unit_end)]
        return add_unit([rows_group(src, dst, sem, base, rows // 8, 8, o, s) for o, s in _offsets(parts)],
                        dst.at[pl.ds(base, rows)])

    u_bwq = [add_unit([bwq_group(u_sem.at[i], i * 256 + g * 32) for g in range(8)], bwq_v.at[pl.ds(i * 256, 256)])
             for i in range(2)]
    u_wq = [add_rows_unit(wq_hbm, wq_v, i * 8192, 8192, PARTS_128) for i in range(2)]
    u_wuk = [add_rows_unit(wuk_hbm, wuk_v, i * 8192, 8192, PARTS_128) for i in range(2)]
    u_ckv = [add_rows_unit(ckv_hbm, ckv_v, i * 2048, 2048, PARTS_512) for i in range(2 * NB)]
    u_wuv = [add_rows_unit(wuv_hbm, wuv_v, i * 8192, 8192, PARTS_128) for i in range(2)]
    u_wo = [add_rows_unit(wo_hbm, wo_v, i * 2048, 2048, PARTS_512) for i in range(2)]
    u_k0 = [add_unit([k0_group(r, i) for i in range(len(PARTS_128))], None) for r in range(NR)]

    row8 = lax.broadcasted_iota(jnp.int32, (8, HD), 0)
    state = {}

    def parity_mask(rows):
        r = lax.broadcasted_iota(jnp.int32, (rows, 2 * DM), 0)
        l = lax.broadcasted_iota(jnp.int32, (rows, 2 * DM), 1)
        return ((r >> 2) & 1) == (l & 1)

    def head_pair(w_ref, j):
        words = w_ref.bitcast(jnp.uint32)[pl.ds(j, DM, stride=NH // 2), :]
        return pltpu.bitcast(words, BF16)

    def load_x(x_ref):
        r = lax.broadcasted_iota(jnp.int32, (8, DM), 0)
        x = jnp.zeros((8, DM), F32)
        for b in range(NB):
            x = jnp.where((r & 3) == b, jnp.broadcast_to(x_ref[b].astype(F32), (8, DM)), x)
        return x.astype(BF16)

    def t_setup():
        for c0 in range(0, DM, 128):
            c = lax.broadcasted_iota(jnp.int32, (128, 2 * DM), 0) + c0
            l = lax.broadcasted_iota(jnp.int32, (128, 2 * DM), 1)
            e_v[pl.ds(c0, 128), :] = jnp.where((l >> 1) == c, 1.0, 0.0).astype(BF16)
        pltpu.make_async_copy(ax_hbm, ax_v, x_sem.at[0]).wait()
        pltpu.make_async_copy(bx_hbm, bx_v, x_sem.at[1]).wait()
        state["xb"] = load_x(bx_v)
        x2 = jnp.dot(load_x(ax_v), e_v[...], preferred_element_type=F32)
        state["xa"] = jnp.where(parity_mask(8), x2, 0.0).astype(BF16)

    def t_qb(half):
        for h in range(half * NH // 2, (half + 1) * NH // 2, 4):
            q = jnp.dot(state["xb"], bwq_v[:, pl.ds(h * HD, 4 * HD)], preferred_element_type=F32)
            for i in range(4):
                qb_v[h + i] = q[:, i * HD:(i + 1) * HD]

    def t_qa(half):
        for j in range(half * 8, half * 8 + 8):
            state["qa", j] = jnp.dot(state["xa"], head_pair(wq_v, j), preferred_element_type=F32).astype(BF16)

    def t_absorb(half):
        mask = parity_mask(8)
        for j in range(half * 8, half * 8 + 8):
            r = lax.dot_general(state["qa", j], head_pair(wuk_v, j), NT, preferred_element_type=F32)
            r_v[pl.ds(8 * j, 8), :] = jnp.where(mask, r, 0.0)

    def permutation(to_batch_major):
        i = lax.broadcasted_iota(jnp.int32, (NB * NH, NB * NH), 0)
        j = lax.broadcasted_iota(jnp.int32, (NB * NH, NB * NH), 1)
        bh, hb = (i, j) if to_batch_major else (j, i)
        return jnp.where(((bh & (NH - 1)) * NB + (bh >> 5)) == hb, 1.0, 0.0).astype(BF16)

    def t_compact():
        q = lax.dot_general(r_v[...].astype(BF16), e_v[...], NT, preferred_element_type=F32)
        qa_v[...] = jnp.dot(permutation(True), q.astype(BF16), preferred_element_type=F32).astype(BF16)

    def t_a_scores(b, half):
        keys = pl.ds(b * SK + half * (SK // 2), SK // 2)
        s = lax.dot_general(qa_v[pl.ds(b * NH, NH), :], ckv_v[keys, :], NT, preferred_element_type=F32)
        sa_v[:, pl.ds(half * (SK // 2), SK // 2)] = s * scale

    def t_a_softmax():
        for g in range(0, NH, 16):
            s = sa_v[pl.ds(g, 16), :]
            p = jnp.exp(s - jnp.max(s, axis=-1, keepdims=True))
            pa_v[pl.ds(g, 16), :] = p.astype(BF16)
            state["la", g] = jnp.sum(p, axis=-1, keepdims=True)

    def t_a_context(b, half):
        keys = pl.ds(b * SK + half * (SK // 2), SK // 2)
        c = jnp.dot(pa_v[:, pl.ds(half * (SK // 2), SK // 2)], ckv_v[keys, :], preferred_element_type=F32)
        if half == 0:
            state["ca"] = c
        else:
            l = jnp.concatenate([state["la", g] for g in range(0, NH, 16)], axis=0)
            cc_v[pl.ds(b * NH, NH), :] = ((state["ca"] + c) / l).astype(BF16)

    def t_expand():
        c = jnp.dot(permutation(False), cc_v[...], preferred_element_type=F32).astype(BF16)
        c2 = jnp.dot(c, e_v[...], preferred_element_type=F32)
        r_v[...] = jnp.where(parity_mask(NB * NH), c2, 0.0)

    def t_up_v(half):
        for j in range(half * 8, half * 8 + 8):
            lhs = r_v[pl.ds(8 * j, 8), :].astype(BF16)
            state["ctx", j] = jnp.dot(lhs, head_pair(wuv_v, j), preferred_element_type=F32)

    def t_out_a(half):
        acc = state.get("oa", jnp.zeros((8, DM), F32))
        for j in range(half * 8, half * 8 + 8):
            ctx = state["ctx", j]
            lhs = jnp.concatenate([jnp.where(row8 < 4, ctx, 0.0), jnp.where(row8 >= 4, ctx, 0.0)], axis=1)
            acc = acc + jnp.dot(lhs.astype(BF16), wo_v[pl.ds(2 * j * HD, 2 * HD), :], preferred_element_type=F32)
        state["oa"] = acc
        if half == 1:
            res = acc + pltpu.roll(acc, 4, 0)
            for b in range(NB):
                out_ref[b, :, pl.ds(0, DM)] = res[b:b + 1, :].astype(out_ref.dtype)

    def b_scores(h, r):
        q = qb_v[h]
        s = None
        for b in range(NB):
            qrow = jnp.where(row8 == b, q, 0.0).astype(BF16)
            d = lax.dot_general(qrow, k_v[r, b], NT, preferred_element_type=F32)
            s = d if s is None else s + d
        sb_v[:, pl.ds(r * KR, KR)] = s * scale

    def b_softmax():
        s = sb_v[...]
        p = jnp.exp(s - jnp.max(s, axis=-1, keepdims=True))
        pb_v[...] = p
        return jnp.sum(p, axis=-1, keepdims=True)

    def b_context(r, acc):
        p = pb_v[:, pl.ds(r * KR, KR)].astype(BF16)
        for b in range(NB):
            d = jnp.dot(p, v_v[r, b], preferred_element_type=F32)
            acc = acc + jnp.where(row8 == b, d, 0.0)
        return acc

    def b_project(h, ctx, l, out):
        row = h * HD if isinstance(h, int) else pl.multiple_of(h * HD, HD)
        return out + jnp.dot((ctx / l).astype(BF16), bwo_v[pl.ds(row, HD), :], preferred_element_type=F32)

    def t_k0(r):
        wait_all(k_v.at[r], k_sem.at[r])
        b_scores(0, r)

    P = functools.partial
    tasks = [(-1, t_setup)]
    tasks += [(u_bwq[1], P(t_qb, i)) for i in range(2)]
    tasks += [(u_wq[1], P(t_qa, i)) for i in range(2)]
    tasks += [(u_wuk[1], P(t_absorb, i)) for i in range(2)] + [(u_wuk[1], t_compact)]
    for b in range(NB):
        tasks += [(u_ckv[2 * b + i], P(t_a_scores, b, i)) for i in range(2)]
        tasks += [(u_ckv[2 * b + 1], t_a_softmax)]
        tasks += [(u_ckv[2 * b + 1], P(t_a_context, b, i)) for i in range(2)]
    tasks += [(u_ckv[-1], t_expand)]
    tasks += [(u_wuv[1], P(t_up_v, i)) for i in range(2)]
    tasks += [(u_wo[1], P(t_out_a, i)) for i in range(2)]
    tasks += [(u_k0[r], P(t_k0, r)) for r in range(NR)]

    issued = [0, 0]

    def issue_until(target):
        while issued[0] < len(stream) and issued[1] < target:
            nbytes, start = stream[issued[0]]
            start()
            issued[0] += 1
            issued[1] += nbytes

    issue_until(1)
    pltpu.make_async_copy(ax_hbm, ax_v, x_sem.at[0]).start()
    pltpu.make_async_copy(bx_hbm, bx_v, x_sem.at[1]).start()
    parts = _offsets(PARTS_128)
    waited = -1
    for i, (need, task) in enumerate(tasks):
        same = [t for t, (n, _) in enumerate(tasks) if n == need]
        later = [n for n, _ in tasks if n > need]
        here = unit_end[need] if need >= 0 else 0
        there = unit_end[later[0]] if later else here
        issue_until(here + LEAD_BYTES + (there - here) * (i - same[0]) // len(same))
        if need in u_k0 and u_k0.index(need) + AHEAD >= NR:
            issue_until(unit_end[-1])
            start_kv(1, 0, u_k0.index(need) + AHEAD - NR, parts)
        while waited < need:
            waited += 1
            if unit_dst[waited] is not None:
                wait_all(unit_dst[waited], u_sem.at[waited])
        task()
    wait_all(bwo_v, bwo_sem)
    l0 = b_softmax()

    def head_step(h, l, out, last_k=False):
        ctx = jnp.zeros((8, HD), F32)
        for r in range(NR):
            nxt, slot = divmod(r + AHEAD, NR)
            hk = None if (last_k and nxt) else h + 1 + nxt
            start_kv(hk, h + nxt, slot, parts[:4])
            wait_all(k_v.at[r], k_sem.at[r])
            b_scores(h + 1, r)
            start_kv(hk, h + nxt, slot, parts[4:])
            wait_all(v_v.at[r], v_sem.at[r])
            ctx = b_context(r, ctx)
        out = b_project(h, ctx, l, out)
        return b_softmax(), out

    l, out = lax.fori_loop(0, NH - 2, lambda h, c: head_step(h, *c), (l0, jnp.zeros((8, DM), F32)))
    l, out = head_step(NH - 2, l, out, last_k=True)
    ctx = jnp.zeros((8, HD), F32)
    for r in range(NR):
        if r + AHEAD < NR:
            start_kv(None, NH - 1, r + AHEAD, parts)
        wait_all(v_v.at[r], v_sem.at[r])
        ctx = b_context(r, ctx)
    out = b_project(NH - 1, ctx, l, out)
    for b in range(NB):
        out_ref[b, :, pl.ds(DM, DM)] = out[b:b + 1, :].astype(out_ref.dtype)


@jax.jit
def pallas_concat_heads__compressed_kv_cla__mha_block_cached__decode_kernel(
    A_x: jax.Array,
    A_c_kv: jax.Array,
    A_w_q: jax.Array,
    A_w_uk: jax.Array,
    A_w_uv: jax.Array,
    A_w_o: jax.Array,
    B_x: jax.Array,
    B_k_cache: jax.Array,
    B_v_cache: jax.Array,
    B_wq: jax.Array,
    B_wo: jax.Array,
):
    assert A_x.shape == (NB, 1, DM) and A_c_kv.shape == (NB, SK, DM) and A_w_q.shape == (DM, NH, HD)
    assert B_x.shape == (NB, 1, DM) and B_k_cache.shape == (NB, NH, SK, HD)
    n_units = 10 + 2 * NB
    scratch = [
        pltpu.VMEM((NB, 1, DM), BF16),
        pltpu.VMEM((NB, 1, DM), BF16),
        pltpu.VMEM((NB * SK, DM), BF16),
        pltpu.VMEM((DM * NH, HD), BF16),
        pltpu.VMEM((DM * NH, HD), BF16),
        pltpu.VMEM((DM * NH, HD), BF16),
        pltpu.VMEM((NH * HD, DM), BF16),
        pltpu.VMEM((DM, NH * HD), BF16),
        pltpu.VMEM((NH * HD, DM), BF16),
        pltpu.VMEM((NR, NB, KR, HD), BF16),
        pltpu.VMEM((NR, NB, KR, HD), BF16),
        pltpu.VMEM((DM, 2 * DM), BF16),
        pltpu.VMEM((NB * NH, 2 * DM), F32),
        pltpu.VMEM((NB * NH, DM), BF16),
        pltpu.VMEM((NH, SK), F32),
        pltpu.VMEM((NH, SK), BF16),
        pltpu.VMEM((NB * NH, DM), BF16),
        pltpu.VMEM((NH, 8, HD), F32),
        pltpu.VMEM((8, SK), F32),
        pltpu.VMEM((8, SK), F32),
        pltpu.SemaphoreType.DMA((2,)),
        pltpu.SemaphoreType.DMA((n_units,)),
        pltpu.SemaphoreType.DMA(()),
        pltpu.SemaphoreType.DMA((NR,)),
        pltpu.SemaphoreType.DMA((NR,)),
    ]
    return pl.pallas_call(
        _kernel,
        out_shape=jax.ShapeDtypeStruct((NB, 1, 2 * DM), A_x.dtype),
        in_specs=[pl.BlockSpec(memory_space=pl.ANY)] * 11,
        out_specs=pl.BlockSpec(memory_space=pltpu.VMEM),
        scratch_shapes=scratch,
        compiler_params=pltpu.CompilerParams(vmem_limit_bytes=100 * MIB),
    )(
        A_x,
        A_c_kv.reshape(NB * SK, DM),
        A_w_q.reshape(DM * NH, HD),
        A_w_uk.reshape(DM * NH, HD),
        A_w_uv.reshape(DM * NH, HD),
        A_w_o.reshape(NH * HD, DM),
        B_x,
        B_k_cache.reshape(NB * NH * SK, HD),
        B_v_cache.reshape(NB * NH * SK, HD),
        B_wq,
        B_wo,
    )
```

```python
import functools

import jax
import jax.numpy as jnp
from jax import lax
import jax.experimental.pallas as pl
import jax.experimental.pallas.tpu as pltpu

F32 = jnp.float32
BF16 = jnp.bfloat16
NT = (((1,), (1,)), ((), ()))

NB, NH, SK, HD, DM = 4, 32, 4096, 128, 512
KR = 1024
NR = SK // KR
AHEAD = 2
PARTS_128 = (144,) * 6 + (160,)
PARTS_512 = (48, 48, 32, 48, 48, 32)
MIB = 1 << 20
LEAD_BYTES = 4 * MIB


def _offsets(parts):
    out, o = [], 0
    for p in parts:
        out.append((o, p))
        o += p
    return out


def _kernel(ax_hbm, ckv_hbm, wq_hbm, wuk_hbm, wuv_hbm, wo_hbm, bx_hbm, k_hbm, v_hbm, bwq_hbm, bwo_hbm,
            out_ref,
            ax_v, bx_v, ckv_v, wq_v, wuk_v, wuv_v, wo_v, bwq_v, bwo_v, k_v, v_v,
            e_v, r_v, qa_v, sa_v, pa_v, cc_v, qb_v, sb_v, pb_v,
            x_sem, u_sem, bwo_sem, k_sem, v_sem):
    scale = HD ** -0.5

    def wait_all(dst, sem):
        pltpu.make_async_copy(dst, dst, sem).wait()

    def rows_group(src, dst, sem, base, stream_rows, n_streams, off, size):
        def start():
            for s in range(n_streams):
                r0 = base + s * stream_rows + off
                pltpu.make_async_copy(src.at[pl.ds(r0, size)], dst.at[pl.ds(r0, size)], sem).start(priority=s % 2)
        return n_streams * size * src.shape[1] * 2, start

    def bwq_group(sem, r0):
        def start():
            for c in range(8):
                sl = (pl.ds(r0 + 16 * (c // 4), 16), pl.ds((c % 4) * 1024, 1024))
                pltpu.make_async_copy(bwq_hbm.at[sl], bwq_v.at[sl], sem).start(priority=c % 2)
        return 8 * 16 * 1024 * 2, start

    def cache_chunk(src, dst, sem, h, r, b, off, size, priority):
        row = (b * NH + h) * SK + r * KR + off
        if not isinstance(row, int):
            row = pl.multiple_of(row, 16)
        pltpu.make_async_copy(src.at[pl.ds(row, size)], dst.at[r, b, pl.ds(off, size)], sem.at[r]).start(priority=priority)

    def start_kv(hk, hv, r, parts):
        for off, size in parts:
            for b in range(NB):
                if hk is not None:
                    cache_chunk(k_hbm, k_v, k_sem, hk, r, b, off, size, 0 if hv is not None else b % 2)
                if hv is not None:
                    cache_chunk(v_hbm, v_v, v_sem, hv, r, b, off, size, 1 if hk is not None else b % 2)

    def k0_group(r, i):
        def start():
            off, size = _offsets(PARTS_128)[i]
            for b in range(NB):
                cache_chunk(k_hbm, k_v, k_sem, 0, r, b, off, size, 0)
                if i < len(PARTS_512):
                    o2, s2 = _offsets(PARTS_512)[i]
                    r0 = r * 1024 + b * 256 + o2
                    pltpu.make_async_copy(bwo_hbm.at[pl.ds(r0, s2)], bwo_v.at[pl.ds(r0, s2)], bwo_sem).start(priority=1)
        return 2 * MIB // len(PARTS_128), start

    stream, unit_end, unit_dst = [], [], []

    def add_unit(groups, dst):
        stream.extend(groups)
        unit_end.append(sum(g[0] for g in stream))
        unit_dst.append(dst)
        return len(unit_end) - 1

    def add_rows_unit(src, dst, base, rows, parts):
        sem = u_sem.at[len(unit_end)]
        return add_unit([rows_group(src, dst, sem, base, rows // 8, 8, o, s) for o, s in _offsets(parts)],
                        dst.at[pl.ds(base, rows)])

    u_bwq = [add_unit([bwq_group(u_sem.at[i], i * 256 + g * 32) for g in range(8)], bwq_v.at[pl.ds(i * 256, 256)])
             for i in range(2)]
    u_wq = [add_rows_unit(wq_hbm, wq_v, i * 8192, 8192, PARTS_128) for i in range(2)]
    u_wuk = [add_rows_unit(wuk_hbm, wuk_v, i * 8192, 8192, PARTS_128) for i in range(2)]
    u_ckv = [add_rows_unit(ckv_hbm, ckv_v, i * 2048, 2048, PARTS_512) for i in range(2 * NB)]
    u_wuv = [add_rows_unit(wuv_hbm, wuv_v, i * 8192, 8192, PARTS_128) for i in range(2)]
    u_wo = [add_rows_unit(wo_hbm, wo_v, i * 2048, 2048, PARTS_512) for i in range(2)]
    u_k0 = [add_unit([k0_group(r, i) for i in range(len(PARTS_128))], None) for r in range(NR)]

    row8 = lax.broadcasted_iota(jnp.int32, (8, HD), 0)
    state = {}

    def parity_mask(rows):
        r = lax.broadcasted_iota(jnp.int32, (rows, 2 * DM), 0)
        l = lax.broadcasted_iota(jnp.int32, (rows, 2 * DM), 1)
        return ((r >> 2) & 1) == (l & 1)

    def head_pair(w_ref, j):
        words = w_ref.bitcast(jnp.uint32)[pl.ds(j, DM, stride=NH // 2), :]
        return pltpu.bitcast(words, BF16)

    def load_x(x_ref):
        x = x_ref[...].astype(F32)
        return jnp.concatenate([x, x], axis=0).astype(BF16)

    def t_setup():
        for c0 in range(0, DM, 128):
            c = lax.broadcasted_iota(jnp.int32, (128, 2 * DM), 0) + c0
            l = lax.broadcasted_iota(jnp.int32, (128, 2 * DM), 1)
            e_v[pl.ds(c0, 128), :] = jnp.where((l >> 1) == c, 1.0, 0.0).astype(BF16)
        pltpu.make_async_copy(ax_hbm, ax_v, x_sem.at[0]).wait()
        pltpu.make_async_copy(bx_hbm, bx_v, x_sem.at[1]).wait()
        state["xb"] = load_x(bx_v)
        x2 = jnp.dot(load_x(ax_v), e_v[...], preferred_element_type=F32)
        state["xa"] = jnp.where(parity_mask(8), x2, 0.0).astype(BF16)

    def t_qb(half):
        for h in range(half * NH // 2, (half + 1) * NH // 2, 4):
            q = jnp.dot(state["xb"], bwq_v[:, pl.ds(h * HD, 4 * HD)], preferred_element_type=F32)
            for i in range(4):
                qb_v[h + i] = q[:, i * HD:(i + 1) * HD]

    def t_qa(half):
        for j in range(half * 8, half * 8 + 8):
            state["qa", j] = jnp.dot(state["xa"], head_pair(wq_v, j), preferred_element_type=F32).astype(BF16)

    def t_absorb(half):
        mask = parity_mask(8)
        for j in range(half * 8, half * 8 + 8):
            r = lax.dot_general(state["qa", j], head_pair(wuk_v, j), NT, preferred_element_type=F32)
            r_v[pl.ds(8 * j, 8), :] = jnp.where(mask, r, 0.0)

    def permutation(to_batch_major):
        i = lax.broadcasted_iota(jnp.int32, (NB * NH, NB * NH), 0)
        j = lax.broadcasted_iota(jnp.int32, (NB * NH, NB * NH), 1)
        bh, hb = (i, j) if to_batch_major else (j, i)
        return jnp.where(((bh & (NH - 1)) * NB + (bh >> 5)) == hb, 1.0, 0.0).astype(BF16)

    def t_compact():
        q = lax.dot_general(r_v[...].astype(BF16), e_v[...], NT, preferred_element_type=F32)
        qa_v[...] = jnp.dot(permutation(True), q.astype(BF16), preferred_element_type=F32).astype(BF16)

    def t_a_scores(b, half):
        keys = pl.ds(b * SK + half * (SK // 2), SK // 2)
        s = lax.dot_general(qa_v[pl.ds(b * NH, NH), :], ckv_v[keys, :], NT, preferred_element_type=F32)
        sa_v[:, pl.ds(half * (SK // 2), SK // 2)] = s * scale

    def t_a_softmax():
        for g in range(0, NH, 16):
            s = sa_v[pl.ds(g, 16), :]
            p = jnp.exp(s - jnp.max(s, axis=-1, keepdims=True))
            pa_v[pl.ds(g, 16), :] = p.astype(BF16)
            state["la", g] = jnp.sum(p, axis=-1, keepdims=True)

    def t_a_context(b, half):
        keys = pl.ds(b * SK + half * (SK // 2), SK // 2)
        c = jnp.dot(pa_v[:, pl.ds(half * (SK // 2), SK // 2)], ckv_v[keys, :], preferred_element_type=F32)
        if half == 0:
            state["ca"] = c
        else:
            l = jnp.concatenate([state["la", g] for g in range(0, NH, 16)], axis=0)
            cc_v[pl.ds(b * NH, NH), :] = ((state["ca"] + c) / l).astype(BF16)

    def t_expand():
        c = jnp.dot(permutation(False), cc_v[...], preferred_element_type=F32).astype(BF16)
        c2 = jnp.dot(c, e_v[...], preferred_element_type=F32)
        r_v[...] = jnp.where(parity_mask(NB * NH), c2, 0.0)

    def t_up_v(half):
        for j in range(half * 8, half * 8 + 8):
            lhs = r_v[pl.ds(8 * j, 8), :].astype(BF16)
            state["ctx", j] = jnp.dot(lhs, head_pair(wuv_v, j), preferred_element_type=F32)

    def t_out_a(half):
        acc = state.get("oa", jnp.zeros((8, DM), F32))
        for j in range(half * 8, half * 8 + 8):
            ctx = state["ctx", j]
            lhs = jnp.concatenate([jnp.where(row8 < 4, ctx, 0.0), jnp.where(row8 >= 4, ctx, 0.0)], axis=1)
            acc = acc + jnp.dot(lhs.astype(BF16), wo_v[pl.ds(2 * j * HD, 2 * HD), :], preferred_element_type=F32)
        state["oa"] = acc
        if half == 1:
            res = acc + pltpu.roll(acc, 4, 0)
            out_ref[:, pl.ds(0, DM)] = res[:NB].astype(out_ref.dtype)

    def b_scores(h, r):
        q = qb_v[h]
        s = None
        for b in range(NB):
            qrow = jnp.where(row8 == b, q, 0.0).astype(BF16)
            d = lax.dot_general(qrow, k_v[r, b], NT, preferred_element_type=F32)
            s = d if s is None else s + d
        sb_v[:, pl.ds(r * KR, KR)] = s * scale

    def b_softmax():
        s = sb_v[...]
        p = jnp.exp(s - jnp.max(s, axis=-1, keepdims=True))
        pb_v[...] = p
        return jnp.sum(p, axis=-1, keepdims=True)

    def b_context(r, acc):
        p = pb_v[:, pl.ds(r * KR, KR)].astype(BF16)
        for b in range(NB):
            d = jnp.dot(p, v_v[r, b], preferred_element_type=F32)
            acc = acc + jnp.where(row8 == b, d, 0.0)
        return acc

    def b_project(h, ctx, l, out):
        row = h * HD if isinstance(h, int) else pl.multiple_of(h * HD, HD)
        return out + jnp.dot((ctx / l).astype(BF16), bwo_v[pl.ds(row, HD), :], preferred_element_type=F32)

    def t_k0(r):
        wait_all(k_v.at[r], k_sem.at[r])
        b_scores(0, r)

    P = functools.partial
    tasks = [(-1, t_setup)]
    tasks += [(u_bwq[1], P(t_qb, i)) for i in range(2)]
    tasks += [(u_wq[1], P(t_qa, i)) for i in range(2)]
    tasks += [(u_wuk[1], P(t_absorb, i)) for i in range(2)] + [(u_wuk[1], t_compact)]
    for b in range(NB):
        tasks += [(u_ckv[2 * b + i], P(t_a_scores, b, i)) for i in range(2)]
        tasks += [(u_ckv[2 * b + 1], t_a_softmax)]
        tasks += [(u_ckv[2 * b + 1], P(t_a_context, b, i)) for i in range(2)]
    tasks += [(u_ckv[-1], t_expand)]
    tasks += [(u_wuv[1], P(t_up_v, i)) for i in range(2)]
    tasks += [(u_wo[1], P(t_out_a, i)) for i in range(2)]
    tasks += [(u_k0[r], P(t_k0, r)) for r in range(NR)]

    issued = [0, 0]

    def issue_until(target):
        while issued[0] < len(stream) and issued[1] < target:
            nbytes, start = stream[issued[0]]
            start()
            issued[0] += 1
            issued[1] += nbytes

    issue_until(1)
    pltpu.make_async_copy(ax_hbm, ax_v, x_sem.at[0]).start()
    pltpu.make_async_copy(bx_hbm, bx_v, x_sem.at[1]).start()
    parts = _offsets(PARTS_128)
    waited = -1
    for i, (need, task) in enumerate(tasks):
        same = [t for t, (n, _) in enumerate(tasks) if n == need]
        later = [n for n, _ in tasks if n > need]
        here = unit_end[need] if need >= 0 else 0
        there = unit_end[later[0]] if later else here
        issue_until(here + LEAD_BYTES + (there - here) * (i - same[0]) // len(same))
        if need in u_k0 and u_k0.index(need) + AHEAD >= NR:
            issue_until(unit_end[-1])
            start_kv(1, 0, u_k0.index(need) + AHEAD - NR, parts)
        while waited < need:
            waited += 1
            if unit_dst[waited] is not None:
                wait_all(unit_dst[waited], u_sem.at[waited])
        task()
    wait_all(bwo_v, bwo_sem)
    l0 = b_softmax()

    def head_step(h, l, out, last_k=False):
        ctx = jnp.zeros((8, HD), F32)
        for r in range(NR):
            nxt, slot = divmod(r + AHEAD, NR)
            hk = None if (last_k and nxt) else h + 1 + nxt
            start_kv(hk, h + nxt, slot, parts[:4])
            wait_all(k_v.at[r], k_sem.at[r])
            b_scores(h + 1, r)
            start_kv(hk, h + nxt, slot, parts[4:])
            wait_all(v_v.at[r], v_sem.at[r])
            ctx = b_context(r, ctx)
        out = b_project(h, ctx, l, out)
        return b_softmax(), out

    l, out = lax.fori_loop(0, NH - 2, lambda h, c: head_step(h, *c), (l0, jnp.zeros((8, DM), F32)))
    l, out = head_step(NH - 2, l, out, last_k=True)
    ctx = jnp.zeros((8, HD), F32)
    for r in range(NR):
        if r + AHEAD < NR:
            start_kv(None, NH - 1, r + AHEAD, parts)
        wait_all(v_v.at[r], v_sem.at[r])
        ctx = b_context(r, ctx)
    out = b_project(NH - 1, ctx, l, out)
    out_ref[:, pl.ds(DM, DM)] = out[:NB].astype(out_ref.dtype)


@jax.jit
def pallas_concat_heads__compressed_kv_cla__mha_block_cached__decode_kernel(
    A_x: jax.Array,
    A_c_kv: jax.Array,
    A_w_q: jax.Array,
    A_w_uk: jax.Array,
    A_w_uv: jax.Array,
    A_w_o: jax.Array,
    B_x: jax.Array,
    B_k_cache: jax.Array,
    B_v_cache: jax.Array,
    B_wq: jax.Array,
    B_wo: jax.Array,
):
    assert A_x.shape == (NB, 1, DM) and A_c_kv.shape == (NB, SK, DM) and A_w_q.shape == (DM, NH, HD)
    assert B_x.shape == (NB, 1, DM) and B_k_cache.shape == (NB, NH, SK, HD)
    n_units = 10 + 2 * NB
    scratch = [
        pltpu.VMEM((NB, DM), BF16),
        pltpu.VMEM((NB, DM), BF16),
        pltpu.VMEM((NB * SK, DM), BF16),
        pltpu.VMEM((DM * NH, HD), BF16),
        pltpu.VMEM((DM * NH, HD), BF16),
        pltpu.VMEM((DM * NH, HD), BF16),
        pltpu.VMEM((NH * HD, DM), BF16),
        pltpu.VMEM((DM, NH * HD), BF16),
        pltpu.VMEM((NH * HD, DM), BF16),
        pltpu.VMEM((NR, NB, KR, HD), BF16),
        pltpu.VMEM((NR, NB, KR, HD), BF16),
        pltpu.VMEM((DM, 2 * DM), BF16),
        pltpu.VMEM((NB * NH, 2 * DM), F32),
        pltpu.VMEM((NB * NH, DM), BF16),
        pltpu.VMEM((NH, SK), F32),
        pltpu.VMEM((NH, SK), BF16),
        pltpu.VMEM((NB * NH, DM), BF16),
        pltpu.VMEM((NH, 8, HD), F32),
        pltpu.VMEM((8, SK), F32),
        pltpu.VMEM((8, SK), F32),
        pltpu.SemaphoreType.DMA((2,)),
        pltpu.SemaphoreType.DMA((n_units,)),
        pltpu.SemaphoreType.DMA(()),
        pltpu.SemaphoreType.DMA((NR,)),
        pltpu.SemaphoreType.DMA((NR,)),
    ]
    out = pl.pallas_call(
        _kernel,
        out_shape=jax.ShapeDtypeStruct((NB, 2 * DM), A_x.dtype),
        in_specs=[pl.BlockSpec(memory_space=pl.ANY)] * 11,
        out_specs=pl.BlockSpec(memory_space=pltpu.VMEM),
        scratch_shapes=scratch,
        compiler_params=pltpu.CompilerParams(vmem_limit_bytes=100 * MIB),
    )(
        A_x.reshape(NB, DM),
        A_c_kv.reshape(NB * SK, DM),
        A_w_q.reshape(DM * NH, HD),
        A_w_uk.reshape(DM * NH, HD),
        A_w_uv.reshape(DM * NH, HD),
        A_w_o.reshape(NH * HD, DM),
        B_x.reshape(NB, DM),
        B_k_cache.reshape(NB * NH * SK, HD),
        B_v_cache.reshape(NB * NH * SK, HD),
        B_wq,
        B_wo,
    )
    return out.reshape(NB, 1, 2 * DM)
```

```python
import jax
import jax.numpy as jnp
from jax import lax
import jax.experimental.pallas as pl
import jax.experimental.pallas.tpu as pltpu

F32 = jnp.float32
BF16 = jnp.bfloat16
NT = (((1,), (1,)), ((), ()))

NB, NH, SK, HD, DM = 4, 32, 4096, 128, 512
KR = 1024
NR = SK // KR
AHEAD = 2
NP = 4
NS = 8
CACHE_CHUNKS = (144,) * 6 + (160,)
NARROW_CHUNKS = (176, 176, 160)
WIDE_CHUNKS = (48, 40, 40)
TAIL_PIECES = ((144, 144, 112, 112), (128, 128), (128, 128))


def _offsets(sizes, start=0):
    out = []
    for size in sizes:
        out.append((start, size))
        start += size
    return out


def _aligned(x, m):
    return x if isinstance(x, int) else pl.multiple_of(x, m)


def _loop(n, body, init=None):
    return lax.fori_loop(0, n, body, init)


def _kernel(ax_hbm, ckv_hbm, wq_hbm, wuk_hbm, wuv_hbm, wo_hbm, bx_hbm, k_hbm, v_hbm, bwq_hbm, bwo_hbm,
            out_ref,
            ax_v, bx_v, ckv_v, wq_v, wuk_v, wuv_v, wo_v, bwq_v, bwo_v, k_v, v_v,
            e_v, pair_v, r_v, qa_v, sa_v, cc_v, qb_v, sb_v, pb_v,
            x_sem, w_sem, ckv_sem, k_sem, v_sem, tail_sem):
    scale = HD ** -0.5
    bwq_sem, wq_sem, wuk_sem, wuv_sem, wo_sem, bwo_sem = (w_sem.at[i] for i in range(6))

    def wait_all(dst, sem):
        pltpu.make_async_copy(dst, dst, sem).wait()

    def start_rows(src, dst, sem, part, base=0, streams=range(NS)):
        chunks = NARROW_CHUNKS if src.shape[1] == HD else WIDE_CHUNKS
        piece = sum(chunks)
        for off, size in _offsets(chunks):
            for s in streams:
                rows = pl.ds(_aligned(base + (s * NP + part) * piece + off, 8), size)
                pltpu.make_async_copy(src.at[rows], dst.at[rows], sem).start(priority=s % 2)

    def start_bwq(part):
        cols = pl.ds(_aligned(part * (NH * HD // NP), HD), NH * HD // NP)
        for off in range(0, DM // NS, 16):
            for s in range(NS):
                rows = pl.ds(s * (DM // NS) + off, 16)
                pltpu.make_async_copy(bwq_hbm.at[rows, cols], bwq_v.at[part, rows], bwq_sem).start(priority=s % 2)

    def cache_copy(src, dst, sem, h, r, b, off, size):
        row = _aligned((b * NH + h) * SK + ((r + b) % NR) * KR + off, 16)
        return pltpu.make_async_copy(src.at[pl.ds(row, size)], dst.at[r, b, pl.ds(off, size)], sem)

    def start_kv(hk, hv, r, chunks=_offsets(CACHE_CHUNKS), sem=None):
        for off, size in chunks:
            for b in range(NB):
                if hk is not None:
                    copy = cache_copy(k_hbm, k_v, k_sem.at[r], hk, r, b, off, size)
                    copy.start(priority=b % 2 if hv is None else 0)
                if hv is not None:
                    copy = cache_copy(v_hbm, v_v, v_sem.at[r] if sem is None else sem, hv, r, b, off, size)
                    copy.start(priority=b % 2 if hk is None else 1)

    row8 = lax.broadcasted_iota(jnp.int32, (8, HD), 0)
    pairs_per_part = NH // 2 // NP

    def parity_mask(rows):
        r = lax.broadcasted_iota(jnp.int32, (rows, 2 * DM), 0)
        l = lax.broadcasted_iota(jnp.int32, (rows, 2 * DM), 1)
        return ((r >> 2) & 1) == (l & 1)

    def head_pair(w_ref, i, k):
        words = w_ref.bitcast(jnp.uint32)
        words = words.at[pl.ds(_aligned(i * pairs_per_part, pairs_per_part), (DM - 1) * NH // 2 + pairs_per_part)]
        return pltpu.bitcast(words[pl.ds(k, DM, stride=NH // 2), :], BF16)

    def permutation(to_batch_major):
        i = lax.broadcasted_iota(jnp.int32, (NB * NH, NB * NH), 0)
        j = lax.broadcasted_iota(jnp.int32, (NB * NH, NB * NH), 1)
        bh, hb = (i, j) if to_batch_major else (j, i)
        return jnp.where((bh % NH) * NB + bh // NH == hb, 1.0, 0.0).astype(BF16)

    def load_x(x_ref):
        x = x_ref[...].astype(F32)
        return jnp.concatenate([x, x], axis=0).astype(BF16)

    x_copies = [pltpu.make_async_copy(ax_hbm, ax_v, x_sem.at[0]), pltpu.make_async_copy(bx_hbm, bx_v, x_sem.at[1])]

    def setup(i, _):
        start_bwq(i)
        c0 = _aligned(i * (DM // NP), DM // NP)
        c = lax.broadcasted_iota(jnp.int32, (DM // NP, 2 * DM), 0) + c0
        l = lax.broadcasted_iota(jnp.int32, (DM // NP, 2 * DM), 1)
        e_v[pl.ds(c0, DM // NP), :] = jnp.where((l >> 1) == c, 1.0, 0.0).astype(BF16)

    _loop(NP, setup)
    for copy in x_copies:
        copy.start()
    _loop(NP, lambda i, _: start_rows(wq_hbm, wq_v, wq_sem, i))
    for copy in x_copies:
        copy.wait()
    xb = load_x(bx_v)
    xa = jnp.dot(load_x(ax_v), e_v[...], preferred_element_type=F32)
    xa = jnp.where(parity_mask(8), xa, 0.0).astype(BF16)

    def b_queries(i, _):
        start_rows(wuk_hbm, wuk_v, wuk_sem, i)
        q = jnp.dot(xb, bwq_v[i], preferred_element_type=F32)
        for k in range(NH // NP):
            qb_v[i * (NH // NP) + k] = q[:, k * HD:(k + 1) * HD]

    wait_all(bwq_v, bwq_sem)
    _loop(NP, b_queries)

    def a_queries(i, _):
        start_rows(ckv_hbm, ckv_v, ckv_sem.at[0], i)
        for k in range(pairs_per_part):
            j = i * pairs_per_part + k
            pair_v[j] = jnp.dot(xa, head_pair(wq_v, i, k), preferred_element_type=F32)

    wait_all(wq_v, wq_sem)
    _loop(NP, a_queries)

    def a_absorb(i, _):
        start_rows(ckv_hbm, ckv_v, ckv_sem.at[1], i, base=SK)
        for k in range(pairs_per_part):
            j = i * pairs_per_part + k
            r = lax.dot_general(pair_v[j].astype(BF16), head_pair(wuk_v, i, k), NT, preferred_element_type=F32)
            r_v[pl.ds(_aligned(8 * j, 8), 8), :] = jnp.where(parity_mask(8), r, 0.0)

    wait_all(wuk_v, wuk_sem)
    _loop(NP, a_absorb)
    q_lat = lax.dot_general(r_v[...].astype(BF16), e_v[...], NT, preferred_element_type=F32)
    qa_v[...] = jnp.dot(permutation(True), q_lat.astype(BF16), preferred_element_type=F32).astype(BF16)

    def a_attention(b, _):
        def start_next(i, streams):
            @pl.when(b + 2 < NB)
            def _():
                start_rows(ckv_hbm, ckv_v, ckv_sem.at[b + 2], i, base=(b + 2) * SK, streams=streams)

            @pl.when(b + 2 == NB)
            def _():
                start_rows(wuv_hbm, wuv_v, wuv_sem, i, streams=streams)

            @pl.when(b + 2 == NB + 1)
            def _():
                start_rows(wo_hbm, wo_v, wo_sem, i, streams=streams)

        def latents(i):
            return ckv_v[pl.ds(_aligned(b * SK + i * (SK // NP), SK // NP), SK // NP), :]

        heads = pl.ds(_aligned(b * NH, NH), NH)

        def scores(i, m):
            start_next(i, range(NS // 2))
            s = lax.dot_general(qa_v[heads, :], latents(i), NT, preferred_element_type=F32) * scale
            sa_v[i] = s
            return jnp.maximum(m, jnp.max(s, axis=-1, keepdims=True))

        def context(i, carry):
            start_next(i, range(NS // 2, NS))
            p = jnp.exp(sa_v[i] - m)
            c = jnp.dot(p.astype(BF16), latents(i), preferred_element_type=F32)
            return carry[0] + c, carry[1] + jnp.sum(p, axis=-1, keepdims=True)

        wait_all(ckv_v.at[pl.ds(_aligned(b * SK, SK), SK)], ckv_sem.at[b])
        m = _loop(NP, scores, jnp.full((NH, 1), -jnp.inf, F32))
        c, l = _loop(NP, context, (jnp.zeros((NH, DM), F32), jnp.zeros((NH, 1), F32)))
        cc_v[heads, :] = (c / l).astype(BF16)

    _loop(NB, a_attention)
    c_lat = jnp.dot(permutation(False), cc_v[...], preferred_element_type=F32).astype(BF16)
    r_v[...] = jnp.where(parity_mask(NB * NH), jnp.dot(c_lat, e_v[...], preferred_element_type=F32), 0.0)

    def a_values(i, _):
        start_rows(bwo_hbm, bwo_v, bwo_sem, i)
        for k in range(pairs_per_part):
            j = i * pairs_per_part + k
            lhs = r_v[pl.ds(_aligned(8 * j, 8), 8), :].astype(BF16)
            pair_v[j] = jnp.dot(lhs, head_pair(wuv_v, i, k), preferred_element_type=F32)

    wait_all(wuv_v, wuv_sem)
    _loop(NP, a_values)

    def a_output(i, acc):
        start_kv(0, None, i)
        for k in range(pairs_per_part):
            j = i * pairs_per_part + k
            ctx = pair_v[j]
            lhs = jnp.concatenate([jnp.where(row8 < NB, ctx, 0.0), jnp.where(row8 >= NB, ctx, 0.0)], axis=1)
            w = wo_v[pl.ds(_aligned(2 * j * HD, 2 * HD), 2 * HD), :]
            acc = acc + jnp.dot(lhs.astype(BF16), w, preferred_element_type=F32)
        return acc

    wait_all(wo_v, wo_sem)
    out_a = _loop(NP, a_output, jnp.zeros((8, DM), F32))
    out_ref[:, pl.ds(0, DM)] = (out_a + pltpu.roll(out_a, NB, 0))[:NB].astype(out_ref.dtype)

    def b_scores(h, r):
        q = qb_v[h]
        s = None
        for b in range(NB):
            d = lax.dot_general(jnp.where(row8 == b, q, 0.0).astype(BF16), k_v[r, b], NT, preferred_element_type=F32)
            s = d if s is None else s + d
        sb_v[r] = s * scale

    def b_softmax():
        s = sb_v[...]
        p = jnp.exp(s - jnp.max(jnp.max(s, axis=0), axis=-1, keepdims=True))
        pb_v[...] = p
        return jnp.sum(jnp.sum(p, axis=0), axis=-1, keepdims=True)

    def b_context(r, acc, off=0, size=KR):
        p = pb_v[r, :, pl.ds(off, size)].astype(BF16)
        for b in range(NB):
            d = jnp.dot(p, v_v[r, b, pl.ds(off, size), :], preferred_element_type=F32)
            acc = acc + jnp.where(row8 == b, d, 0.0)
        return acc

    def b_project(h, ctx, l, out):
        w = bwo_v[pl.ds(_aligned(h * HD, HD), HD), :]
        return out + jnp.dot((ctx / l).astype(BF16), w, preferred_element_type=F32)

    def first_scores(r, _):
        @pl.when(r + AHEAD >= NR)
        def _():
            start_kv(1, 0, r + AHEAD - NR)

        wait_all(k_v.at[r], k_sem.at[r])
        b_scores(0, r)

    _loop(NR, first_scores)
    wait_all(bwo_v, bwo_sem)

    def head_step(h, carry):
        l, out = carry
        ctx = jnp.zeros((8, HD), F32)
        for r in range(NR):
            nxt, slot = divmod(r + AHEAD, NR)

            def start(chunks):
                if nxt:
                    pl.when(h + 2 < NH)(lambda: start_kv(h + 2, h + 1, slot, chunks))
                    pl.when(h + 2 == NH)(lambda: start_kv(None, NH - 1, slot, chunks))
                else:
                    start_kv(h + 1, h, slot, chunks)

            start(_offsets(CACHE_CHUNKS)[:4])
            wait_all(k_v.at[r], k_sem.at[r])
            b_scores(h + 1, r)
            start(_offsets(CACHE_CHUNKS)[4:])
            wait_all(v_v.at[r], v_sem.at[r])
            ctx = b_context(r, ctx)
        out = b_project(h, ctx, l, out)
        return b_softmax(), out

    l, out = _loop(NH - 1, head_step, (b_softmax(), jnp.zeros((8, DM), F32)))

    pieces, off = [], 0
    for sizes in TAIL_PIECES:
        pieces.append((off, sum(sizes), _offsets(sizes, off)))
        off += sum(sizes)
    ctx = jnp.zeros((8, HD), F32)
    for r in range(NR - 1):
        if r + AHEAD < NR - 1:
            start_kv(None, NH - 1, r + AHEAD)
        elif r + AHEAD == NR - 1:
            for i, (_, _, chunks) in enumerate(pieces):
                start_kv(None, NH - 1, NR - 1, chunks, tail_sem.at[i])
        wait_all(v_v.at[r], v_sem.at[r])
        ctx = b_context(r, ctx)
    for i, (o, size, _) in enumerate(pieces):
        wait_all(v_v.at[NR - 1, :, pl.ds(o, size)], tail_sem.at[i])
        ctx = b_context(NR - 1, ctx, o, size)
    out = b_project(NH - 1, ctx, l, out)
    out_ref[:, pl.ds(DM, DM)] = out[:NB].astype(out_ref.dtype)


@jax.jit
def pallas_concat_heads__compressed_kv_cla__mha_block_cached__decode_kernel(
    A_x: jax.Array,
    A_c_kv: jax.Array,
    A_w_q: jax.Array,
    A_w_uk: jax.Array,
    A_w_uv: jax.Array,
    A_w_o: jax.Array,
    B_x: jax.Array,
    B_k_cache: jax.Array,
    B_v_cache: jax.Array,
    B_wq: jax.Array,
    B_wo: jax.Array,
):
    assert A_x.shape == (NB, 1, DM) and A_c_kv.shape == (NB, SK, DM) and A_w_q.shape == (DM, NH, HD)
    assert B_x.shape == (NB, 1, DM) and B_k_cache.shape == (NB, NH, SK, HD)
    scratch = [
        pltpu.VMEM((NB, DM), BF16),
        pltpu.VMEM((NB, DM), BF16),
        pltpu.VMEM((NB * SK, DM), BF16),
        pltpu.VMEM((DM * NH, HD), BF16),
        pltpu.VMEM((DM * NH, HD), BF16),
        pltpu.VMEM((DM * NH, HD), BF16),
        pltpu.VMEM((NH * HD, DM), BF16),
        pltpu.VMEM((NP, DM, NH * HD // NP), BF16),
        pltpu.VMEM((NH * HD, DM), BF16),
        pltpu.VMEM((NR, NB, KR, HD), BF16),
        pltpu.VMEM((NR, NB, KR, HD), BF16),
        pltpu.VMEM((DM, 2 * DM), BF16),
        pltpu.VMEM((NH // 2, 8, HD), F32),
        pltpu.VMEM((NB * NH, 2 * DM), F32),
        pltpu.VMEM((NB * NH, DM), BF16),
        pltpu.VMEM((NP, NH, SK // NP), F32),
        pltpu.VMEM((NB * NH, DM), BF16),
        pltpu.VMEM((NH, 8, HD), F32),
        pltpu.VMEM((NR, 8, KR), F32),
        pltpu.VMEM((NR, 8, KR), F32),
        pltpu.SemaphoreType.DMA((2,)),
        pltpu.SemaphoreType.DMA((6,)),
        pltpu.SemaphoreType.DMA((NB,)),
        pltpu.SemaphoreType.DMA((NR,)),
        pltpu.SemaphoreType.DMA((NR,)),
        pltpu.SemaphoreType.DMA((len(TAIL_PIECES),)),
    ]
    out = pl.pallas_call(
        _kernel,
        out_shape=jax.ShapeDtypeStruct((NB, 2 * DM), A_x.dtype),
        in_specs=[pl.BlockSpec(memory_space=pl.ANY)] * 11,
        out_specs=pl.BlockSpec(memory_space=pltpu.VMEM),
        scratch_shapes=scratch,
        compiler_params=pltpu.CompilerParams(vmem_limit_bytes=100 * 1024 * 1024),
    )(
        A_x.reshape(NB, DM),
        A_c_kv.reshape(NB * SK, DM),
        A_w_q.reshape(DM * NH, HD),
        A_w_uk.reshape(DM * NH, HD),
        A_w_uv.reshape(DM * NH, HD),
        A_w_o.reshape(NH * HD, DM),
        B_x.reshape(NB, DM),
        B_k_cache.reshape(NB * NH * SK, HD),
        B_v_cache.reshape(NB * NH * SK, HD),
        B_wq,
        B_wo,
    )
    return out.reshape(NB, 1, 2 * DM)
```

```python
import jax
import jax.numpy as jnp
from jax import lax
import jax.experimental.pallas as pl
import jax.experimental.pallas.tpu as pltpu

F32 = jnp.float32
BF16 = jnp.bfloat16
NT = (((1,), (1,)), ((), ()))

NB, NH, SK, HD, DM = 4, 32, 4096, 128, 512
KR = 1024
NR = SK // KR
AHEAD = 2
NP = 4
NS = 8
CHUNK = 32 * 1024
SHIFT = dict(ckv=0, wq=0, wuk=0, wuv=0, wo=0, k=16384, v=16384, bwq=16384, bwo=16384)
TAIL_PIECES = (512, 256, 256)
FIRST = 4
RANGE_ROT = (0, 2, 0, 2)
K_ROT = (0, 0, 0, 0)
V_ROT = (0, 0, 0, 0)
ROW_ROT = (0,) * 8


def _aligned(x, m):
    return x if isinstance(x, int) else pl.multiple_of(x, m)


def _loop(n, body, init=None):
    return lax.fori_loop(0, n, body, init)


def _kernel(ax_hbm, ckv_hbm, wq_hbm, wuk_hbm, wuv_hbm, wo_hbm, bx_hbm, k_hbm, v_hbm, bwq_hbm, bwo_hbm,
            out_ref,
            ax_v, bx_v, ckv_v, wq_v, wuk_v, wuv_v, wo_v, bwq_v, bwo_v, k_v, v_v,
            words_v, e_v, pair_v, r_v, qa_v, sa_v, cc_v, qb_v, sb_v, pb_v,
            x_sem, w_sem, ckv_sem, k_sem, v_sem, tail_sem):
    scale = HD ** -0.5
    bwq_sem, wq_sem, wuk_sem, wuv_sem, wo_sem, bwo_sem = (w_sem.at[i] for i in range(6))

    def wait_all(dst, sem):
        pltpu.make_async_copy(dst, dst, sem).wait()

    def row_chunks(src, name, rows, split_last):
        step, shift = CHUNK // (2 * src.shape[1]), SHIFT[name] // (2 * src.shape[1])
        chunks = [[(off, step)] for off in range(0, rows, step)]
        if split_last and shift:
            chunks[-1] = [(rows - step, step - shift), (rows - shift, shift)]
        return shift, chunks

    def start_rows(name, src, dst, sem, part, base=0, streams=range(NS)):
        total = DM * NH * HD // src.shape[1]
        piece = total // (NS * NP)
        for c in range(piece * 2 * src.shape[1] // CHUNK):
            for s in streams:
                shift, chunks = row_chunks(src, name, piece, s == NS - 1)
                for off, size in chunks[(c + ROW_ROT[s]) % len(chunks)]:
                    row = shift + (s * NP + part) * piece + off
                    rows = pl.ds(_aligned(base + (row % total if s == NS - 1 else row), 8), size)
                    pltpu.make_async_copy(src.at[rows], dst.at[rows], sem).start(priority=s % 2)

    def start_bwq(part):
        cols = pl.ds(_aligned(part * (NH * HD // NP), HD), NH * HD // NP)
        for off in range(0, DM // NS, 16):
            for s in range(NS):
                rows = pl.ds(s * (DM // NS) + off, 16)
                pltpu.make_async_copy(bwq_hbm.at[rows, cols], bwq_v.at[part, rows], bwq_sem).start(priority=s % 2)

    def start_cache(name, src, dst, sem, h, r, b, c, priority):
        key_range = (r + RANGE_ROT[b]) % NR
        shift, chunks = row_chunks(src, "k", KR, not isinstance(r, int) or key_range == NR - 1)
        for off, size in chunks[c]:
            row = _aligned((b * NH + h) * SK + (shift + key_range * KR + off) % SK, 8)
            pltpu.make_async_copy(src.at[pl.ds(row, size)], dst.at[r, b, pl.ds(off, size)], sem).start(priority=priority)

    slot_chunks = range(KR * 2 * HD // CHUNK)

    def start_kv(hk, hv, r, chunks=slot_chunks, sem=None):
        for c in chunks:
            for b in range(NB):
                if hk is not None:
                    start_cache("k", k_hbm, k_v, k_sem.at[r], hk, r, b, (c + K_ROT[b]) % len(slot_chunks), b % 2 if hv is None else 0)
                if hv is not None:
                    start_cache("v", v_hbm, v_v, v_sem.at[r] if sem is None else sem, hv, r, b,
                                (c + V_ROT[b]) % len(slot_chunks) if sem is None else c, b % 2 if hk is None else 1)

    row8 = lax.broadcasted_iota(jnp.int32, (8, HD), 0)
    pairs_per_part = NH // 2 // NP

    def parity_mask(rows):
        r = lax.broadcasted_iota(jnp.int32, (rows, 2 * DM), 0)
        l = lax.broadcasted_iota(jnp.int32, (rows, 2 * DM), 1)
        return ((r >> 2) & 1) == (l & 1)

    def for_head_pairs(w_ref, start_part, body):
        def to_words(i, _):
            rows = DM * NH // NP
            w = w_ref[pl.ds(_aligned(i * rows, rows), rows), :]
            words_v[pl.ds(_aligned(i * rows // 2, rows // 2), rows // 2), :] = pltpu.bitcast(w, jnp.uint32)

        def eight_pairs(i, _):
            window = words_v.at[pl.ds(_aligned(8 * i, 8), DM * NH // 2 + 8)]
            for k in range(8):
                if k % pairs_per_part == 0:
                    start_part(i * (8 // pairs_per_part) + k // pairs_per_part)
                body(8 * i + k, pltpu.bitcast(window[pl.ds(k, DM, stride=NH // 2), :], BF16))

        _loop(NP, to_words)
        _loop(NH // 16, eight_pairs)

    def permutation(to_batch_major):
        i = lax.broadcasted_iota(jnp.int32, (NB * NH, NB * NH), 0)
        j = lax.broadcasted_iota(jnp.int32, (NB * NH, NB * NH), 1)
        bh, hb = (i, j) if to_batch_major else (j, i)
        return jnp.where((bh % NH) * NB + bh // NH == hb, 1.0, 0.0).astype(BF16)

    def load_x(x_ref):
        x = x_ref[...].astype(F32)
        return jnp.concatenate([x, x], axis=0).astype(BF16)

    x_copies = [pltpu.make_async_copy(ax_hbm, ax_v, x_sem.at[0]), pltpu.make_async_copy(bx_hbm, bx_v, x_sem.at[1])]

    def setup(i, _):
        start_bwq(i)
        c0 = _aligned(i * (DM // NP), DM // NP)
        c = lax.broadcasted_iota(jnp.int32, (DM // NP, 2 * DM), 0) + c0
        l = lax.broadcasted_iota(jnp.int32, (DM // NP, 2 * DM), 1)
        e_v[pl.ds(c0, DM // NP), :] = jnp.where((l >> 1) == c, 1.0, 0.0).astype(BF16)

    _loop(NP, setup)
    for copy in x_copies:
        copy.start()
    _loop(NP, lambda i, _: start_rows("wq", wq_hbm, wq_v, wq_sem, i))
    for copy in x_copies:
        copy.wait()
    xb = load_x(bx_v)
    xa = jnp.dot(load_x(ax_v), e_v[...], preferred_element_type=F32)
    xa = jnp.where(parity_mask(8), xa, 0.0).astype(BF16)

    def b_queries(i, _):
        start_rows("wuk", wuk_hbm, wuk_v, wuk_sem, i)
        q = jnp.dot(xb, bwq_v[i], preferred_element_type=F32)
        for k in range(NH // NP):
            qb_v[i * (NH // NP) + k] = q[:, k * HD:(k + 1) * HD]

    wait_all(bwq_v, bwq_sem)
    _loop(NP, b_queries)

    def a_queries(j, w):
        pair_v[j] = jnp.dot(xa, w, preferred_element_type=F32)

    wait_all(wq_v, wq_sem)
    for_head_pairs(wq_v, lambda i: start_rows("ckv", ckv_hbm, ckv_v, ckv_sem.at[0], i), a_queries)

    def a_absorb(j, w):
        r = lax.dot_general(pair_v[j].astype(BF16), w, NT, preferred_element_type=F32)
        r_v[pl.ds(_aligned(8 * j, 8), 8), :] = jnp.where(parity_mask(8), r, 0.0)

    wait_all(wuk_v, wuk_sem)
    for_head_pairs(wuk_v, lambda i: start_rows("ckv", ckv_hbm, ckv_v, ckv_sem.at[1], i, base=SK), a_absorb)
    q_lat = lax.dot_general(r_v[...].astype(BF16), e_v[...], NT, preferred_element_type=F32)
    qa_v[...] = jnp.dot(permutation(True), q_lat.astype(BF16), preferred_element_type=F32).astype(BF16)

    def a_attention(b, _):
        def start_next(i, streams):
            @pl.when(b + 2 < NB)
            def _():
                start_rows("ckv", ckv_hbm, ckv_v, ckv_sem.at[b + 2], i, base=(b + 2) * SK, streams=streams)

            @pl.when(b + 2 == NB)
            def _():
                start_rows("wuv", wuv_hbm, wuv_v, wuv_sem, i, streams=streams)

            @pl.when(b + 2 == NB + 1)
            def _():
                start_rows("wo", wo_hbm, wo_v, wo_sem, i, streams=streams)

        def latents(i):
            return ckv_v[pl.ds(_aligned(b * SK + i * (SK // NP), SK // NP), SK // NP), :]

        heads = pl.ds(_aligned(b * NH, NH), NH)

        def scores(i, m):
            start_next(i, range(NS // 2))
            s = lax.dot_general(qa_v[heads, :], latents(i), NT, preferred_element_type=F32) * scale
            sa_v[i] = s
            return jnp.maximum(m, jnp.max(s, axis=-1, keepdims=True))

        def context(i, carry):
            start_next(i, range(NS // 2, NS))
            p = jnp.exp(sa_v[i] - m)
            c = jnp.dot(p.astype(BF16), latents(i), preferred_element_type=F32)
            return carry[0] + c, carry[1] + jnp.sum(p, axis=-1, keepdims=True)

        wait_all(ckv_v.at[pl.ds(_aligned(b * SK, SK), SK)], ckv_sem.at[b])
        m = _loop(NP, scores, jnp.full((NH, 1), -jnp.inf, F32))
        c, l = _loop(NP, context, (jnp.zeros((NH, DM), F32), jnp.zeros((NH, 1), F32)))
        cc_v[heads, :] = (c / l).astype(BF16)

    _loop(NB, a_attention)
    c_lat = jnp.dot(permutation(False), cc_v[...], preferred_element_type=F32).astype(BF16)
    r_v[...] = jnp.where(parity_mask(NB * NH), jnp.dot(c_lat, e_v[...], preferred_element_type=F32), 0.0)

    def a_values(j, w):
        lhs = r_v[pl.ds(_aligned(8 * j, 8), 8), :].astype(BF16)
        pair_v[j] = jnp.dot(lhs, w, preferred_element_type=F32)

    wait_all(wuv_v, wuv_sem)
    for_head_pairs(wuv_v, lambda i: start_rows("bwo", bwo_hbm, bwo_v, bwo_sem, i), a_values)

    def a_output(i, acc):
        start_kv(0, None, i)
        for k in range(pairs_per_part):
            j = i * pairs_per_part + k
            ctx = pair_v[j]
            lhs = jnp.concatenate([jnp.where(row8 < NB, ctx, 0.0), jnp.where(row8 >= NB, ctx, 0.0)], axis=1)
            w = wo_v[pl.ds(_aligned(2 * j * HD, 2 * HD), 2 * HD), :]
            acc = acc + jnp.dot(lhs.astype(BF16), w, preferred_element_type=F32)
        return acc

    wait_all(wo_v, wo_sem)
    out_a = _loop(NP, a_output, jnp.zeros((8, DM), F32))
    out_ref[:, pl.ds(0, DM)] = (out_a + pltpu.roll(out_a, NB, 0))[:NB].astype(out_ref.dtype)

    def b_scores(h, r):
        q = qb_v[h].astype(BF16)
        row = lax.broadcasted_iota(jnp.int32, (8, KR), 0)
        s = None
        for b in range(NB):
            d = lax.dot_general(q, k_v[r, b], NT, preferred_element_type=F32)
            s = d if s is None else jnp.where(row == b, d, s)
        sb_v[r] = s * scale

    def b_softmax():
        s = sb_v[...]
        p = jnp.exp(s - jnp.max(jnp.max(s, axis=0), axis=-1, keepdims=True))
        pb_v[...] = p
        return jnp.sum(jnp.sum(p, axis=0), axis=-1, keepdims=True)

    def b_context(r, acc, off=0, size=KR):
        p = pb_v[r, :, pl.ds(off, size)].astype(BF16)
        for b in range(NB):
            d = jnp.dot(p, v_v[r, b, pl.ds(off, size), :], preferred_element_type=F32)
            acc = acc + jnp.where(row8 == b, d, 0.0)
        return acc

    def b_project(h, ctx, l, out):
        w = bwo_v[pl.ds(_aligned(h * HD, HD), HD), :]
        return out + jnp.dot((ctx / l).astype(BF16), w, preferred_element_type=F32)

    def first_scores(r, _):
        @pl.when(r + AHEAD >= NR)
        def _():
            start_kv(1, 0, r + AHEAD - NR)

        wait_all(k_v.at[r], k_sem.at[r])
        b_scores(0, r)

    _loop(NR, first_scores)
    wait_all(bwo_v, bwo_sem)

    def head_step(h, carry):
        l, out = carry
        ctx = jnp.zeros((8, HD), F32)
        for r in range(NR):
            nxt, slot = divmod(r + AHEAD, NR)

            def start(chunks):
                if nxt:
                    pl.when(h + 2 < NH)(lambda: start_kv(h + 2, h + 1, slot, chunks))
                    pl.when(h + 2 == NH)(lambda: start_kv(None, NH - 1, slot, chunks))
                else:
                    start_kv(h + 1, h, slot, chunks)

            start(slot_chunks[:FIRST])
            wait_all(k_v.at[r], k_sem.at[r])
            b_scores(h + 1, r)
            start(slot_chunks[FIRST:])
            wait_all(v_v.at[r], v_sem.at[r])
            ctx = b_context(r, ctx)
        out = b_project(h, ctx, l, out)
        return b_softmax(), out

    l, out = _loop(NH - 1, head_step, (b_softmax(), jnp.zeros((8, DM), F32)))

    keys_per_chunk = CHUNK // (2 * HD)
    pieces = [(sum(TAIL_PIECES[:i]), size) for i, size in enumerate(TAIL_PIECES)]
    ctx = jnp.zeros((8, HD), F32)
    for r in range(NR - 1):
        if r + AHEAD < NR - 1:
            start_kv(None, NH - 1, r + AHEAD)
        elif r + AHEAD == NR - 1:
            for i, (off, size) in enumerate(pieces):
                chunks = slot_chunks[off // keys_per_chunk:(off + size) // keys_per_chunk]
                start_kv(None, NH - 1, NR - 1, chunks, tail_sem.at[i])
        wait_all(v_v.at[r], v_sem.at[r])
        ctx = b_context(r, ctx)
    for i, (off, size) in enumerate(pieces):
        wait_all(v_v.at[NR - 1, :, pl.ds(off, size)], tail_sem.at[i])
        ctx = b_context(NR - 1, ctx, off, size)
    out = b_project(NH - 1, ctx, l, out)
    out_ref[:, pl.ds(DM, DM)] = out[:NB].astype(out_ref.dtype)


@jax.jit
def pallas_concat_heads__compressed_kv_cla__mha_block_cached__decode_kernel(
    A_x: jax.Array,
    A_c_kv: jax.Array,
    A_w_q: jax.Array,
    A_w_uk: jax.Array,
    A_w_uv: jax.Array,
    A_w_o: jax.Array,
    B_x: jax.Array,
    B_k_cache: jax.Array,
    B_v_cache: jax.Array,
    B_wq: jax.Array,
    B_wo: jax.Array,
):
    assert A_x.shape == (NB, 1, DM) and A_c_kv.shape == (NB, SK, DM) and A_w_q.shape == (DM, NH, HD)
    assert B_x.shape == (NB, 1, DM) and B_k_cache.shape == (NB, NH, SK, HD)
    scratch = [
        pltpu.VMEM((NB, DM), BF16),
        pltpu.VMEM((NB, DM), BF16),
        pltpu.VMEM((NB * SK, DM), BF16),
        pltpu.VMEM((DM * NH, HD), BF16),
        pltpu.VMEM((DM * NH, HD), BF16),
        pltpu.VMEM((DM * NH, HD), BF16),
        pltpu.VMEM((NH * HD, DM), BF16),
        pltpu.VMEM((NP, DM, NH * HD // NP), BF16),
        pltpu.VMEM((NH * HD, DM), BF16),
        pltpu.VMEM((NR, NB, KR, HD), BF16),
        pltpu.VMEM((NR, NB, KR, HD), BF16),
        pltpu.VMEM((DM * NH // 2 + 16, HD), jnp.uint32),
        pltpu.VMEM((DM, 2 * DM), BF16),
        pltpu.VMEM((NH // 2, 8, HD), F32),
        pltpu.VMEM((NB * NH, 2 * DM), F32),
        pltpu.VMEM((NB * NH, DM), BF16),
        pltpu.VMEM((NP, NH, SK // NP), F32),
        pltpu.VMEM((NB * NH, DM), BF16),
        pltpu.VMEM((NH, 8, HD), F32),
        pltpu.VMEM((NR, 8, KR), F32),
        pltpu.VMEM((NR, 8, KR), F32),
        pltpu.SemaphoreType.DMA((2,)),
        pltpu.SemaphoreType.DMA((6,)),
        pltpu.SemaphoreType.DMA((NB,)),
        pltpu.SemaphoreType.DMA((NR,)),
        pltpu.SemaphoreType.DMA((NR,)),
        pltpu.SemaphoreType.DMA((len(TAIL_PIECES),)),
    ]
    out = pl.pallas_call(
        _kernel,
        out_shape=jax.ShapeDtypeStruct((NB, 2 * DM), A_x.dtype),
        in_specs=[pl.BlockSpec(memory_space=pl.ANY)] * 11,
        out_specs=pl.BlockSpec(memory_space=pltpu.VMEM),
        scratch_shapes=scratch,
        compiler_params=pltpu.CompilerParams(vmem_limit_bytes=100 * 1024 * 1024),
    )(
        A_x.reshape(NB, DM),
        A_c_kv.reshape(NB * SK, DM),
        A_w_q.reshape(DM * NH, HD),
        A_w_uk.reshape(DM * NH, HD),
        A_w_uv.reshape(DM * NH, HD),
        A_w_o.reshape(NH * HD, DM),
        B_x.reshape(NB, DM),
        B_k_cache.reshape(NB * NH * SK, HD),
        B_v_cache.reshape(NB * NH * SK, HD),
        B_wq,
        B_wo,
    )
    return out.reshape(NB, 1, 2 * DM)
```

```python
import jax
import jax.numpy as jnp
from jax import lax
import jax.experimental.pallas as pl
import jax.experimental.pallas.tpu as pltpu

F32 = jnp.float32
BF16 = jnp.bfloat16
NT = (((1,), (1,)), ((), ()))

NB, NH, SK, HD, DM = 4, 32, 4096, 128, 512
KR = 1024
NR = SK // KR
AHEAD = 2
NP = 4
NS = 8
STREAM_ORDER = (0, 7, 1, 6, 2, 5, 3, 4)
CHUNK = 32 * 1024
SHIFT = dict(ckv=0, wq=0, wuk=0, wuv=0, wo=0, cache=16384, bwo=16384)
TAIL_PIECES = (512, 256, 256)


def _aligned(x, m):
    return x if isinstance(x, int) else pl.multiple_of(x, m)


def _loop(n, body, init=None):
    return lax.fori_loop(0, n, body, init)


def _kernel(ax_hbm, ckv_hbm, wq_hbm, wuk_hbm, wuv_hbm, wo_hbm, bx_hbm, k_hbm, v_hbm, bwq_hbm, bwo_hbm,
            out_ref,
            ax_v, bx_v, ckv_v, wq_v, wuk_v, wuv_v, wo_v, bwq_v, bwo_v, k_v, v_v,
            words_v, e_v, pair_v, r_v, qa_v, sa_v, cc_v, qb_v, sb_v, pb_v,
            x_sem, w_sem, ckv_sem, k_sem, v_sem, tail_sem):
    scale = HD ** -0.5
    bwq_sem, wq_sem, wuk_sem, wuv_sem, wo_sem, bwo_sem = (w_sem.at[i] for i in range(6))

    def wait_all(dst, sem):
        pltpu.make_async_copy(dst, dst, sem).wait()

    def row_chunks(src, name, rows, split_last):
        step, shift = CHUNK // (2 * src.shape[1]), SHIFT[name] // (2 * src.shape[1])
        chunks = [[(off, step)] for off in range(0, rows, step)]
        if split_last and shift:
            chunks[-1] = [(rows - step, step - shift), (rows - shift, shift)]
        return shift, chunks

    def start_rows(name, src, dst, sem, part, base=0, streams=range(NS)):
        total = DM * NH * HD // src.shape[1]
        piece = total // (NS * NP)
        for c in range(piece * 2 * src.shape[1] // CHUNK):
            for n in streams:
                s = STREAM_ORDER[n]
                shift, chunks = row_chunks(src, name, piece, s == NS - 1)
                for off, size in chunks[c]:
                    row = shift + (s * NP + part) * piece + off
                    rows = pl.ds(_aligned(base + (row % total if s == NS - 1 else row), 8), size)
                    pltpu.make_async_copy(src.at[rows], dst.at[rows], sem).start(priority=n % 2)

    def start_bwq(part):
        cols = pl.ds(_aligned(part * (NH * HD // NP), HD), NH * HD // NP)
        for off in range(0, DM // NS, 16):
            for s in range(NS):
                rows = pl.ds(s * (DM // NS) + off, 16)
                pltpu.make_async_copy(bwq_hbm.at[rows, cols], bwq_v.at[part, rows], bwq_sem).start(priority=s % 2)

    def start_cache(src, dst, sem, h, r, b, c, priority):
        key_range = (r + 2 * b) % NR
        shift, chunks = row_chunks(src, "cache", KR, not isinstance(r, int) or key_range == NR - 1)
        for off, size in chunks[c]:
            row = _aligned((b * NH + h) * SK + (shift + key_range * KR + off) % SK, 8)
            pltpu.make_async_copy(src.at[pl.ds(row, size)], dst.at[r, b, pl.ds(off, size)], sem).start(priority=priority)

    slot_chunks = range(KR * 2 * HD // CHUNK)

    def start_kv(hk, hv, r, chunks=slot_chunks):
        for c in chunks:
            for b in range(NB):
                start_cache(k_hbm, k_v, k_sem.at[r], hk, r, b, c, 0)
                start_cache(v_hbm, v_v, v_sem.at[r], hv, r, b, c, 1)

    def start_alone(src, dst, sem, h, r, chunks=slot_chunks):
        for i in range(len(chunks)):
            for b in range(NB):
                start_cache(src, dst, sem, h, r, b, chunks[(i + b) % len(chunks)], b % 2)

    row8 = lax.broadcasted_iota(jnp.int32, (8, HD), 0)
    pairs_per_part = NH // 2 // NP

    def parity_mask(rows):
        r = lax.broadcasted_iota(jnp.int32, (rows, 2 * DM), 0)
        l = lax.broadcasted_iota(jnp.int32, (rows, 2 * DM), 1)
        return ((r >> 2) & 1) == (l & 1)

    def for_head_pairs(w_ref, start_part, body):
        def to_words(i, _):
            rows = DM * NH // NP
            w = w_ref[pl.ds(_aligned(i * rows, rows), rows), :]
            words_v[pl.ds(_aligned(i * rows // 2, rows // 2), rows // 2), :] = pltpu.bitcast(w, jnp.uint32)

        def eight_pairs(i, _):
            window = words_v.at[pl.ds(_aligned(8 * i, 8), DM * NH // 2 + 8)]
            for k in range(8):
                if k % pairs_per_part == 0:
                    start_part(i * (8 // pairs_per_part) + k // pairs_per_part)
                body(8 * i + k, pltpu.bitcast(window[pl.ds(k, DM, stride=NH // 2), :], BF16))

        _loop(NP, to_words)
        _loop(NH // 16, eight_pairs)

    def permutation(to_batch_major):
        i = lax.broadcasted_iota(jnp.int32, (NB * NH, NB * NH), 0)
        j = lax.broadcasted_iota(jnp.int32, (NB * NH, NB * NH), 1)
        bh, hb = (i, j) if to_batch_major else (j, i)
        return jnp.where((bh % NH) * NB + bh // NH == hb, 1.0, 0.0).astype(BF16)

    def load_x(x_ref):
        x = x_ref[...].astype(F32)
        return jnp.concatenate([x, x], axis=0).astype(BF16)

    x_copies = [pltpu.make_async_copy(ax_hbm, ax_v, x_sem.at[0]), pltpu.make_async_copy(bx_hbm, bx_v, x_sem.at[1])]

    def setup(i, _):
        start_bwq(i)
        c0 = _aligned(i * (DM // NP), DM // NP)
        c = lax.broadcasted_iota(jnp.int32, (DM // NP, 2 * DM), 0) + c0
        l = lax.broadcasted_iota(jnp.int32, (DM // NP, 2 * DM), 1)
        e_v[pl.ds(c0, DM // NP), :] = jnp.where((l >> 1) == c, 1.0, 0.0).astype(BF16)

    _loop(NP, setup)
    for copy in x_copies:
        copy.start()
    _loop(NP, lambda i, _: start_rows("wq", wq_hbm, wq_v, wq_sem, i))
    for copy in x_copies:
        copy.wait()
    xb = load_x(bx_v)
    xa = jnp.dot(load_x(ax_v), e_v[...], preferred_element_type=F32)
    xa = jnp.where(parity_mask(8), xa, 0.0).astype(BF16)

    def b_queries(i, _):
        start_rows("wuk", wuk_hbm, wuk_v, wuk_sem, i)
        q = jnp.dot(xb, bwq_v[i], preferred_element_type=F32)
        for k in range(NH // NP):
            qb_v[i * (NH // NP) + k] = q[:, k * HD:(k + 1) * HD]

    wait_all(bwq_v, bwq_sem)
    _loop(NP, b_queries)

    def a_queries(j, w):
        pair_v[j] = jnp.dot(xa, w, preferred_element_type=F32)

    wait_all(wq_v, wq_sem)
    for_head_pairs(wq_v, lambda i: start_rows("ckv", ckv_hbm, ckv_v, ckv_sem.at[0], i), a_queries)

    def a_absorb(j, w):
        r = lax.dot_general(pair_v[j].astype(BF16), w, NT, preferred_element_type=F32)
        r_v[pl.ds(_aligned(8 * j, 8), 8), :] = jnp.where(parity_mask(8), r, 0.0)

    wait_all(wuk_v, wuk_sem)
    for_head_pairs(wuk_v, lambda i: start_rows("ckv", ckv_hbm, ckv_v, ckv_sem.at[1], i, base=SK), a_absorb)
    q_lat = lax.dot_general(r_v[...].astype(BF16), e_v[...], NT, preferred_element_type=F32)
    qa_v[...] = jnp.dot(permutation(True), q_lat.astype(BF16), preferred_element_type=F32).astype(BF16)

    def a_attention(b, _):
        def start_next(i, streams):
            @pl.when(b + 2 < NB)
            def _():
                start_rows("ckv", ckv_hbm, ckv_v, ckv_sem.at[b + 2], i, base=(b + 2) * SK, streams=streams)

            @pl.when(b + 2 == NB)
            def _():
                start_rows("wuv", wuv_hbm, wuv_v, wuv_sem, i, streams=streams)

            @pl.when(b + 2 == NB + 1)
            def _():
                start_rows("wo", wo_hbm, wo_v, wo_sem, i, streams=streams)

        def latents(i):
            return ckv_v[pl.ds(_aligned(b * SK + i * (SK // NP), SK // NP), SK // NP), :]

        heads = pl.ds(_aligned(b * NH, NH), NH)

        def scores(i, m):
            start_next(i, range(NS // 2))
            s = lax.dot_general(qa_v[heads, :], latents(i), NT, preferred_element_type=F32) * scale
            sa_v[i] = s
            return jnp.maximum(m, jnp.max(s, axis=-1, keepdims=True))

        def context(i, carry):
            start_next(i, range(NS // 2, NS))
            p = jnp.exp(sa_v[i] - m)
            c = jnp.dot(p.astype(BF16), latents(i), preferred_element_type=F32)
            return carry[0] + c, carry[1] + jnp.sum(p, axis=-1, keepdims=True)

        wait_all(ckv_v.at[pl.ds(_aligned(b * SK, SK), SK)], ckv_sem.at[b])
        m = _loop(NP, scores, jnp.full((NH, 1), -jnp.inf, F32))
        c, l = _loop(NP, context, (jnp.zeros((NH, DM), F32), jnp.zeros((NH, 1), F32)))
        cc_v[heads, :] = (c / l).astype(BF16)

    _loop(NB, a_attention)
    c_lat = jnp.dot(permutation(False), cc_v[...], preferred_element_type=F32).astype(BF16)
    r_v[...] = jnp.where(parity_mask(NB * NH), jnp.dot(c_lat, e_v[...], preferred_element_type=F32), 0.0)

    def a_values(j, w):
        lhs = r_v[pl.ds(_aligned(8 * j, 8), 8), :].astype(BF16)
        pair_v[j] = jnp.dot(lhs, w, preferred_element_type=F32)

    wait_all(wuv_v, wuv_sem)
    for_head_pairs(wuv_v, lambda i: start_rows("bwo", bwo_hbm, bwo_v, bwo_sem, i), a_values)

    def a_output(i, acc):
        start_alone(k_hbm, k_v, k_sem.at[i], 0, i)
        for k in range(pairs_per_part):
            j = i * pairs_per_part + k
            ctx = pair_v[j]
            lhs = jnp.concatenate([jnp.where(row8 < NB, ctx, 0.0), jnp.where(row8 >= NB, ctx, 0.0)], axis=1)
            w = wo_v[pl.ds(_aligned(2 * j * HD, 2 * HD), 2 * HD), :]
            acc = acc + jnp.dot(lhs.astype(BF16), w, preferred_element_type=F32)
        return acc

    wait_all(wo_v, wo_sem)
    out_a = _loop(NP, a_output, jnp.zeros((8, DM), F32))
    out_ref[:, pl.ds(0, DM)] = (out_a + pltpu.roll(out_a, NB, 0))[:NB].astype(out_ref.dtype)

    def b_scores(h, r):
        q = qb_v[h].astype(BF16)
        row = lax.broadcasted_iota(jnp.int32, (8, KR), 0)
        s = None
        for b in range(NB):
            d = lax.dot_general(q, k_v[r, b], NT, preferred_element_type=F32)
            s = d if s is None else jnp.where(row == b, d, s)
        sb_v[r] = s * scale

    def b_softmax():
        s = sb_v[...]
        p = jnp.exp(s - jnp.max(jnp.max(s, axis=0), axis=-1, keepdims=True))
        pb_v[...] = p
        return jnp.sum(jnp.sum(p, axis=0), axis=-1, keepdims=True)

    def b_context(r, acc, off=0, size=KR):
        p = pb_v[r, :, pl.ds(off, size)].astype(BF16)
        for b in range(NB):
            d = jnp.dot(p, v_v[r, b, pl.ds(off, size), :], preferred_element_type=F32)
            acc = acc + jnp.where(row8 == b, d, 0.0)
        return acc

    def b_project(h, ctx, l, out):
        w = bwo_v[pl.ds(_aligned(h * HD, HD), HD), :]
        return out + jnp.dot((ctx / l).astype(BF16), w, preferred_element_type=F32)

    def first_scores(r, _):
        @pl.when(r + AHEAD >= NR)
        def _():
            start_kv(1, 0, r + AHEAD - NR)

        wait_all(k_v.at[r], k_sem.at[r])
        b_scores(0, r)

    _loop(NR, first_scores)
    wait_all(bwo_v, bwo_sem)

    def head_step(h, carry):
        l, out = carry
        ctx = jnp.zeros((8, HD), F32)
        for r in range(NR):
            nxt, slot = divmod(r + AHEAD, NR)

            def start(chunks):
                if nxt:
                    pl.when(h + 2 < NH)(lambda: start_kv(h + 2, h + 1, slot, chunks))
                    pl.when(h + 2 == NH)(lambda: start_alone(v_hbm, v_v, v_sem.at[slot], NH - 1, slot, chunks))
                else:
                    start_kv(h + 1, h, slot, chunks)

            start(slot_chunks[:4])
            wait_all(k_v.at[r], k_sem.at[r])
            b_scores(h + 1, r)
            start(slot_chunks[4:])
            wait_all(v_v.at[r], v_sem.at[r])
            ctx = b_context(r, ctx)
        out = b_project(h, ctx, l, out)
        return b_softmax(), out

    l, out = _loop(NH - 1, head_step, (b_softmax(), jnp.zeros((8, DM), F32)))

    keys_per_chunk = CHUNK // (2 * HD)
    pieces = [(sum(TAIL_PIECES[:i]), size) for i, size in enumerate(TAIL_PIECES)]
    ctx = jnp.zeros((8, HD), F32)
    for r in range(NR - 1):
        if r + AHEAD < NR - 1:
            start_alone(v_hbm, v_v, v_sem.at[r + AHEAD], NH - 1, r + AHEAD)
        elif r + AHEAD == NR - 1:
            for i, (off, size) in enumerate(pieces):
                chunks = slot_chunks[off // keys_per_chunk:(off + size) // keys_per_chunk]
                start_alone(v_hbm, v_v, tail_sem.at[i], NH - 1, NR - 1, chunks)
        wait_all(v_v.at[r], v_sem.at[r])
        ctx = b_context(r, ctx)
    for i, (off, size) in enumerate(pieces):
        wait_all(v_v.at[NR - 1, :, pl.ds(off, size)], tail_sem.at[i])
        ctx = b_context(NR - 1, ctx, off, size)
    out = b_project(NH - 1, ctx, l, out)
    out_ref[:, pl.ds(DM, DM)] = out[:NB].astype(out_ref.dtype)


@jax.jit
def pallas_concat_heads__compressed_kv_cla__mha_block_cached__decode_kernel(
    A_x: jax.Array,
    A_c_kv: jax.Array,
    A_w_q: jax.Array,
    A_w_uk: jax.Array,
    A_w_uv: jax.Array,
    A_w_o: jax.Array,
    B_x: jax.Array,
    B_k_cache: jax.Array,
    B_v_cache: jax.Array,
    B_wq: jax.Array,
    B_wo: jax.Array,
):
    assert A_x.shape == (NB, 1, DM) and A_c_kv.shape == (NB, SK, DM) and A_w_q.shape == (DM, NH, HD)
    assert B_x.shape == (NB, 1, DM) and B_k_cache.shape == (NB, NH, SK, HD)
    scratch = [
        pltpu.VMEM((NB, DM), BF16),
        pltpu.VMEM((NB, DM), BF16),
        pltpu.VMEM((NB * SK, DM), BF16),
        pltpu.VMEM((DM * NH, HD), BF16),
        pltpu.VMEM((DM * NH, HD), BF16),
        pltpu.VMEM((DM * NH, HD), BF16),
        pltpu.VMEM((NH * HD, DM), BF16),
        pltpu.VMEM((NP, DM, NH * HD // NP), BF16),
        pltpu.VMEM((NH * HD, DM), BF16),
        pltpu.VMEM((NR, NB, KR, HD), BF16),
        pltpu.VMEM((NR, NB, KR, HD), BF16),
        pltpu.VMEM((DM * NH // 2 + 16, HD), jnp.uint32),
        pltpu.VMEM((DM, 2 * DM), BF16),
        pltpu.VMEM((NH // 2, 8, HD), F32),
        pltpu.VMEM((NB * NH, 2 * DM), F32),
        pltpu.VMEM((NB * NH, DM), BF16),
        pltpu.VMEM((NP, NH, SK // NP), F32),
        pltpu.VMEM((NB * NH, DM), BF16),
        pltpu.VMEM((NH, 8, HD), F32),
        pltpu.VMEM((NR, 8, KR), F32),
        pltpu.VMEM((NR, 8, KR), F32),
        pltpu.SemaphoreType.DMA((2,)),
        pltpu.SemaphoreType.DMA((6,)),
        pltpu.SemaphoreType.DMA((NB,)),
        pltpu.SemaphoreType.DMA((NR,)),
        pltpu.SemaphoreType.DMA((NR,)),
        pltpu.SemaphoreType.DMA((len(TAIL_PIECES),)),
    ]
    out = pl.pallas_call(
        _kernel,
        out_shape=jax.ShapeDtypeStruct((NB, 2 * DM), A_x.dtype),
        in_specs=[pl.BlockSpec(memory_space=pl.ANY)] * 11,
        out_specs=pl.BlockSpec(memory_space=pltpu.VMEM),
        scratch_shapes=scratch,
        compiler_params=pltpu.CompilerParams(vmem_limit_bytes=100 * 1024 * 1024),
    )(
        A_x.reshape(NB, DM),
        A_c_kv.reshape(NB * SK, DM),
        A_w_q.reshape(DM * NH, HD),
        A_w_uk.reshape(DM * NH, HD),
        A_w_uv.reshape(DM * NH, HD),
        A_w_o.reshape(NH * HD, DM),
        B_x.reshape(NB, DM),
        B_k_cache.reshape(NB * NH * SK, HD),
        B_v_cache.reshape(NB * NH * SK, HD),
        B_wq,
        B_wo,
    )
    return out.reshape(NB, 1, 2 * DM)
```
